```python
import os as _os
_os.environ.setdefault("JAX_PLATFORMS", "cpu")
import jax
import jax.numpy as jnp

def _softmax(x, axis=-1):
    return jax.nn.softmax(x, axis=axis)
def _gelu(x):
    return jax.nn.gelu(x, approximate=True)
def _silu(x):
    return jax.nn.silu(x)
def _sigmoid(x):
    return jax.nn.sigmoid(x)
def _layernorm(x, axis=-1, eps=1e-5):
    m = jnp.mean(x, axis=axis, keepdims=True)
    v = jnp.var(x, axis=axis, keepdims=True)
    return (x - m) / jnp.sqrt(v + eps)
def _scatter_add(tgt, idx, src, axis=0):
    return tgt.at[idx].add(src)
def _segment_sum(src, seg, n):
    return jax.ops.segment_sum(src, seg, n)
class _Rng:
    def __init__(self, key):
        self._k = key
    def _next(self):
        self._k, sub = jax.random.split(self._k)
        return sub
    def normal(self, shape):
        return jax.random.normal(self._next(), shape, dtype=jnp.bfloat16)
    def randint(self, lo, hi, shape):
        return jax.random.randint(self._next(), shape, lo, hi, dtype=jnp.int32)
    def uniform(self, shape, lo=0.0, hi=1.0):
        return jax.random.uniform(self._next(), shape, jnp.bfloat16, lo, hi)
    def permutation(self, n):
        return jax.random.permutation(self._next(), n)


kernel_name = 'standalone__dense_activation_silu__prompt'

def setup_inputs():
    _rng = _Rng(jax.random.key(int.from_bytes(__import__("os").urandom(4), "little")))
    _w = (lambda a: (lambda t: t.astype(jnp.bfloat16) if jnp.issubdtype(t.dtype, jnp.floating) else t)(jnp.asarray(a)))
    B, S, D, F = 1, 2048, 448, 1792
    return {
        "x": _w((lambda *s: _rng.normal(s) * 0.05)(B, S, D)),
        "w1": _w((lambda *s: _rng.normal(s) * 0.05)(D, F) * (D ** -0.5)),
        "w2": _w((lambda *s: _rng.normal(s) * 0.05)(F, D) * (F ** -0.5)),
    }

def reference(x, w1, w2):
    h = jnp.einsum("bsd,df->bsf", x, w1)
    h = _silu(h)
    out = jnp.einsum("bsf,fd->bsd", h, w2)
    return out
```

```python
import jax
import jax.numpy as jnp
import jax.experimental.pallas as pl
import jax.experimental.pallas.tpu as pltpu

U = 128

_LOADS = (
    (("x", 0, 2), ("w1", 0, 2)),
    (("x", 2, 3), ("w1", 2, 3)),
    (("x", 3, 5), ("w1", 3, 5)),
    (("x", 5, 10), ("w1", 5, 9)),
    (("w1", 9, 14), ("w2", 0, 14), ("x", 10, 16)),
)
_PROG = (
    ("wait", 0), ("T", 0, 2), ("mm1", 0, 2, 0, 2),
    ("wait", 1), ("mm1", 2, 3, 0, 2), ("T", 2, 3), ("mm1", 0, 3, 2, 3),
    ("wait", 2), ("mm1", 3, 5, 0, 3), ("T", 3, 5), ("mm1", 0, 5, 3, 5),
    ("wait", 3), ("mm1", 5, 10, 0, 5), ("T", 5, 9), ("mm1", 0, 10, 5, 9),
    ("wait", 4), ("mm1", 10, 16, 0, 9), ("T", 9, 14), ("mm1", 0, 16, 9, 14),
    ("mm2", 0, 4), ("mm2", 4, 8), ("mm2", 8, 12), ("mm2", 12, 14), ("mm2", 14, 16),
)


def _silu(h):
    return h * pltpu.reciprocal(1.0 + jnp.exp(-h), approx=True)


def _kernel(xT_hbm, w1_hbm, w2T_hbm, oT_hbm,
            x_v, w1_v, w2_v, w1T_v, o_v, in_sem, out_sem, bar_sem):
    src = {"x": xT_hbm, "w1": w1_hbm, "w2": w2T_hbm}
    dst = {"x": x_v, "w1": w1_v, "w2": w2_v}
    nf = w1_hbm.shape[1] // U

    def in_cp(g, entry):
        name, u0, u1 = entry
        sl = pl.ds(u0 * U, (u1 - u0) * U)
        return pltpu.make_async_copy(src[name].at[:, sl], dst[name].at[:, sl], in_sem.at[g])

    def out_cp(i0, i1):
        sl = pl.ds(i0 * U, (i1 - i0) * U)
        return pltpu.make_async_copy(o_v.at[:, sl], oT_hbm.at[:, sl], out_sem.at[0])

    for g, group in enumerate(_LOADS):
        for entry in group:
            in_cp(g, entry).start()
        if g + 1 < len(_LOADS):
            pl.semaphore_signal(bar_sem, 1)
            pl.semaphore_wait(bar_sem, 1)

    act = {}
    outs = []
    for op in _PROG:
        if op[0] == "wait":
            for entry in _LOADS[op[1]]:
                in_cp(op[1], entry).wait()
        elif op[0] == "T":
            for j in range(op[1], op[2]):
                w1T_v[j * U:(j + 1) * U, :] = w1_v[:, j * U:(j + 1) * U].T
        elif op[0] == "mm1":
            _, i0, i1, j0, j1 = op
            h = jnp.dot(w1T_v[j0 * U:j1 * U, :], x_v[:, i0 * U:i1 * U],
                        preferred_element_type=jnp.float32)
            a = _silu(h).astype(jnp.bfloat16)
            for i in range(i0, i1):
                for j in range(j0, j1):
                    act[i, j] = a[(j - j0) * U:(j - j0 + 1) * U, (i - i0) * U:(i - i0 + 1) * U]
        else:
            _, i0, i1 = op
            a = jnp.concatenate(
                [jnp.concatenate([act[i, j] for i in range(i0, i1)], axis=1) for j in range(nf)],
                axis=0)
            o = jnp.dot(w2_v[...], a, preferred_element_type=jnp.float32)
            o_v[:, i0 * U:i1 * U] = o.astype(o_v.dtype)
            out_cp(i0, i1).start()
            outs.append((i0, i1))
    for i0, i1 in outs:
        out_cp(i0, i1).wait()


@jax.jit
def pallas_standalone__dense_activation_silu__prompt_kernel(
    x: jax.Array,
    w1: jax.Array,
    w2: jax.Array,
):
    B, S, D = x.shape
    F = w1.shape[1]
    M = B * S
    assert (M, D, F) == (2048, 448, 1792)
    oT = pl.pallas_call(
        _kernel,
        in_specs=[pl.BlockSpec(memory_space=pl.ANY)] * 3,
        out_specs=pl.BlockSpec(memory_space=pl.ANY),
        out_shape=jax.ShapeDtypeStruct((D, M), x.dtype),
        scratch_shapes=[
            pltpu.VMEM((D, M + U), x.dtype),
            pltpu.VMEM((D, F), w1.dtype),
            pltpu.VMEM((D, F), w2.dtype),
            pltpu.VMEM((F, D), w1.dtype),
            pltpu.VMEM((D, M + U), x.dtype),
            pltpu.SemaphoreType.DMA((len(_LOADS),)),
            pltpu.SemaphoreType.DMA((1,)),
            pltpu.SemaphoreType.REGULAR,
        ],
        compiler_params=pltpu.CompilerParams(vmem_limit_bytes=100 * 1024 * 1024),
    )(x.reshape(M, D).T, w1, w2.T)
    return oT.T.reshape(B, S, D)
```

```python
import jax
import jax.numpy as jnp
import jax.experimental.pallas as pl
import jax.experimental.pallas.tpu as pltpu

U = 128
D, F, S = 448, 1792, 2048
NF, NS = F // U, S // U
KB = (0, 128, 256, 384, 448)
KP = (0, 128, 256, 384, 512)
NK = 4
NSEM = 4

_GROUPS = (
    (("w1", 0, 4, 0, 1),),
    (("x", 0, 4, 0, 1),),
    (("x", 4, 8, 0, 1),),
    (("w1", 4, 8, 0, 1),),
    (("x", 8, 12, 0, 1),),
    (("w1", 0, 4, 1, 4), ("x", 0, 4, 1, 4)),
    (("w1", 4, 8, 1, 4), ("x", 4, 8, 1, 4)),
    (("w1", 8, 14, 0, 4), ("x", 8, 12, 1, 4)),
    (("x", 12, 16, 0, 4), ("w2", 0, 14, 0, 4)),
)

_PROG = (
    ("wait", 0), ("T", 0, 4, 0, 1),
    ("wait", 1), ("mm1", 0, 4, 0, 4, 0, 1), ("keep", 0, 4, 0, 2),
    ("wait", 2), ("keep", 0, 4, 2, 4), ("mm1", 4, 8, 0, 4, 0, 1), ("keep", 4, 8, 0, 1),
    ("wait", 3), ("T", 4, 8, 0, 1), ("keep", 4, 8, 1, 4),
    ("mm1", 0, 8, 4, 8, 0, 1), ("keep", 0, 8, 4, 6),
    ("wait", 4), ("keep", 0, 8, 6, 8), ("mm1", 8, 12, 0, 8, 0, 1), ("keep", 8, 12, 0, 4),
    ("wait", 5), ("T", 0, 4, 1, 4), ("keep", 8, 12, 4, 8), ("mm1", 0, 4, 0, 4, 1, 4),
    ("wait", 6), ("T", 4, 8, 1, 4), ("mm1", 4, 8, 0, 4, 1, 4),
    ("wait", 7), ("T", 8, 14, 0, 4), ("mm1", 0, 8, 4, 8, 1, 4), ("mm1", 8, 12, 0, 8, 1, 4),
    ("mm1", 0, 12, 8, 14, 0, 4),
    ("wait", 8), ("mm1", 12, 16, 0, 14, 0, 4),
    ("mm2", 0, 4, 0, D), ("mm2", 4, 8, 0, D), ("mm2", 8, 12, 0, D), ("mm2", 12, 14, 0, D),
    ("mm2", 14, 16, 0, 160), ("mm2", 14, 16, 160, 304), ("mm2", 14, 16, 304, D),
)

_BASE = {"x": 0, "w1": NS * D, "w2": (NS + NF) * D}
_W1T_BASE = (NS + 2 * NF) * D
_KEEP_BASE = _W1T_BASE + NK * NF * U
_KEEP_SLOT = {}
for _op in _PROG:
    if _op[0] == "keep":
        for _i in range(_op[1], _op[2]):
            for _j in range(_op[3], _op[4]):
                _KEEP_SLOT[_i, _j] = len(_KEEP_SLOT)
_BUF_ROWS = _KEEP_BASE + 2 * U * len(_KEEP_SLOT)


def _silu(h):
    return h * pltpu.reciprocal(1.0 + jnp.exp(-h), approx=True)


def _kernel(xT_hbm, w1_hbm, w2T_hbm, oT_hbm, buf, o_buf, sems):
    hbm = {"x": xT_hbm, "w1": w1_hbm, "w2": w2T_hbm}
    buf32 = buf.bitcast(jnp.uint32)
    o_buf32 = o_buf.bitcast(jnp.uint32)

    def load(r0, r1):
        return pltpu.bitcast(buf32[r0 // 2:r1 // 2, :], jnp.bfloat16)

    def store(ref32, r0, val):
        ref32[r0 // 2:(r0 + val.shape[0]) // 2, :] = pltpu.bitcast(val, jnp.uint32)

    def load_k(name, u, k0, k1):
        base = _BASE[name] + u * D
        val = load(base + KB[k0], base + KB[k1])
        if k1 == NK:
            val = jnp.concatenate([val, jnp.zeros((KP[NK] - D, U), val.dtype)], axis=0)
        return val

    def w1t_row(j, k):
        return _W1T_BASE + (k * NF + j) * U

    def keep_rows(i, j):
        r = _KEEP_BASE // 2 + _KEEP_SLOT[i, j] * U
        return slice(r, r + U)

    def in_copies(g):
        return [
            pltpu.make_async_copy(
                hbm[name].at[KB[k0]:KB[k1], u * U:(u + 1) * U],
                buf.at[_BASE[name] + u * D + KB[k0]:_BASE[name] + u * D + KB[k1], :],
                sems.at[g % NSEM])
            for name, u0, u1, k0, k1 in _GROUPS[g] for u in range(u0, u1)
        ]

    for g in range(NSEM):
        for cp in in_copies(g):
            cp.start()

    partial, act, out_copies = {}, {}, []
    for op in _PROG:
        if op[0] == "wait":
            g = op[1]
            for cp in in_copies(g):
                cp.wait()
            if g + NSEM < len(_GROUPS):
                for cp in in_copies(g + NSEM):
                    cp.start()
        elif op[0] == "T":
            _, j0, j1, k0, k1 = op
            for j in range(j0, j1):
                t = load_k("w1", j, k0, k1).T
                for k in range(k0, k1):
                    store(buf32, w1t_row(j, k), t[:, KP[k] - KP[k0]:KP[k + 1] - KP[k0]])
        elif op[0] == "mm1":
            _, i0, i1, j0, j1, k0, k1 = op
            lhs = jnp.concatenate(
                [jnp.concatenate([load(w1t_row(j, k), w1t_row(j, k) + U) for k in range(k0, k1)],
                                 axis=1) for j in range(j0, j1)], axis=0)
            rhs = jnp.concatenate([load_k("x", i, k0, k1) for i in range(i0, i1)], axis=1)
            h = jnp.dot(lhs, rhs, preferred_element_type=jnp.float32)
            if k0 > 0:
                h = h + jnp.concatenate(
                    [jnp.concatenate([pltpu.bitcast(buf32[keep_rows(i, j), :], jnp.float32)
                                      for i in range(i0, i1)], axis=1) for j in range(j0, j1)],
                    axis=0)
            dest = partial
            if k1 == NK:
                h, dest = _silu(h).astype(jnp.bfloat16), act
            for i in range(i0, i1):
                for j in range(j0, j1):
                    dest[i, j] = h[(j - j0) * U:(j - j0 + 1) * U, (i - i0) * U:(i - i0 + 1) * U]
        elif op[0] == "keep":
            _, i0, i1, j0, j1 = op
            for j in range(j0, j1):
                for i in range(i0, i1):
                    buf32[keep_rows(i, j), :] = pltpu.bitcast(partial[i, j], jnp.uint32)
        else:
            _, i0, i1, r0, r1 = op
            lhs = jnp.concatenate(
                [load(_BASE["w2"] + j * D + r0, _BASE["w2"] + j * D + r1) for j in range(NF)],
                axis=1)
            rhs = jnp.concatenate(
                [jnp.concatenate([act[i, j] for i in range(i0, i1)], axis=1) for j in range(NF)],
                axis=0)
            o = jnp.dot(lhs, rhs, preferred_element_type=jnp.float32).astype(jnp.bfloat16)
            for i in range(i0, i1):
                store(o_buf32, i * D + r0, o[:, (i - i0) * U:(i - i0 + 1) * U])
            for i in range(i0, i1):
                cp = pltpu.make_async_copy(o_buf.at[i * D + r0:i * D + r1, :],
                                           oT_hbm.at[r0:r1, i * U:(i + 1) * U], sems.at[0])
                cp.start()
                out_copies.append(cp)
    for cp in out_copies:
        cp.wait()


@jax.jit
def pallas_standalone__dense_activation_silu__prompt_kernel(
    x: jax.Array,
    w1: jax.Array,
    w2: jax.Array,
):
    assert x.shape == (1, S, D) and w1.shape == (D, F) and w2.shape == (F, D)
    assert x.dtype == w1.dtype == w2.dtype == jnp.bfloat16
    flags = {"XLA_TPU_RESCHEDULE_DMA_DONES": True} if jax.__version_info__ >= (0, 12) else None
    out_t = pl.pallas_call(
        _kernel,
        in_specs=[pl.BlockSpec(memory_space=pl.ANY)] * 3,
        out_specs=pl.BlockSpec(memory_space=pl.ANY),
        out_shape=jax.ShapeDtypeStruct((D, S), x.dtype),
        scratch_shapes=[
            pltpu.VMEM((_BUF_ROWS, U), jnp.bfloat16),
            pltpu.VMEM((NS * D, U), jnp.bfloat16),
            pltpu.SemaphoreType.DMA((NSEM,)),
        ],
        compiler_params=pltpu.CompilerParams(vmem_limit_bytes=100 * 1024 * 1024, flags=flags),
    )(x.reshape(S, D).T, w1, w2.T)
    return out_t.T.reshape(1, S, D)
```

```python
import jax
import jax.numpy as jnp
import jax.experimental.pallas as pl
import jax.experimental.pallas.tpu as pltpu

U = 128
D, F, S = 448, 1792, 2048
NF, NS = F // U, S // U
NK = 4
KB = (0, 128, 256, 384, 448)
KP = (0, 128, 256, 384, 512)
REM, MAIN, ALL = (3, 4), (0, 3), (0, 4)
NSEM = 3

_GROUPS = (
    (("w1", 0, 4, *REM),),
    (("x", 0, 4, *REM),),
    (("x", 4, 8, *REM), ("w1", 4, 8, *REM)),
    (("x", 8, NS, *REM),),
    (("w1", 0, 4, *MAIN), ("x", 0, 4, *MAIN)),
    (("w1", 4, 8, *MAIN), ("x", 4, 8, *MAIN)),
    (("w1", 8, NF, *ALL), ("x", 8, NS, *MAIN)),
    (("w2", 0, NF, *ALL),),
)

_PROG = (
    ("wait", 0), ("T", 0, 4, *REM),
    ("wait", 1), ("mm1", 0, 4, 0, 4, *REM), ("pin", 3, 0),
    ("wait", 2), ("T", 4, 8, *REM), ("mm1", 4, 8, 0, 4, *REM), ("mm1", 0, 8, 4, 8, *REM),
    ("pin", 7, 5),
    ("wait", 3), ("mm1", 8, NS, 0, 8, *REM), ("pin", NS - 1, 2),
    ("wait", 4), ("T", 0, 4, *MAIN), ("mm1", 0, 4, 0, 4, *MAIN),
    ("wait", 5), ("T", 4, 8, *MAIN), ("mm1", 4, 8, 0, 4, *MAIN),
    ("wait", 6), ("T", 8, NF, *ALL), ("mm1", 0, 8, 4, 8, *MAIN), ("mm1", 8, NS, 0, 8, *MAIN),
    ("mm1", 0, NS, 8, NF, *ALL),
    ("wait", 7),
    ("mm2", 0, 4, 0, D), ("mm2", 4, 8, 0, D), ("mm2", 8, 12, 0, D), ("mm2", 12, 14, 0, D),
    ("mm2", 14, 15, 0, D), ("mm2", 15, NS, 0, D // 2), ("mm2", 15, NS, D // 2, D),
)

_BASE = {"x": 0, "w1": NS, "w2": NS + NF, "w1T": NS + 2 * NF}
_BASE["pin"] = _BASE["w1T"] + pl.cdiv(NK * NF, 3)
_BUF_UNITS = (_BASE["pin"] + 1) | 1


def _silu(h):
    return h * pltpu.reciprocal(1.0 + jnp.exp(-h), approx=True)


def _kernel(xT_hbm, w1_hbm, w2T_hbm, oT_hbm, buf, o_buf, sems):
    hbm = {"x": xT_hbm, "w1": w1_hbm, "w2": w2T_hbm}

    def cols(name, u0, u1):
        return slice((_BASE[name] + u0) * U, (_BASE[name] + u1) * U)

    def w1t_block(j, k):
        unit, slot = divmod(k * NF + j, 3)
        return slice(slot * U, (slot + 1) * U), cols("w1T", unit, unit + 1)

    def load_k(name, u0, u1, k0, k1):
        val = buf[KB[k0]:KB[k1], cols(name, u0, u1)]
        if k1 == NK:
            zeros = jnp.zeros((KP[NK] - D, val.shape[1]), val.dtype)
            val = jnp.concatenate([val, zeros], axis=0)
        return val

    def in_copies(g):
        return [
            pltpu.make_async_copy(
                hbm[name].at[KB[k0]:KB[k1], u0 * U:u1 * U],
                buf.at[KB[k0]:KB[k1], cols(name, u0, u1)],
                sems.at[g % NSEM])
            for name, u0, u1, k0, k1 in _GROUPS[g]
        ]

    def gather(tiles, i0, i1, j0, j1):
        return jnp.concatenate(
            [jnp.concatenate([tiles[i, j] for i in range(i0, i1)], axis=1)
             for j in range(j0, j1)], axis=0)

    for g in range(NSEM):
        for cp in in_copies(g):
            cp.start()

    hid = {}
    k_done = {}
    out_copies = []
    for op in _PROG:
        if op[0] == "wait":
            g = op[1]
            for cp in in_copies(g):
                cp.wait()
            if g + NSEM < len(_GROUPS):
                for cp in in_copies(g + NSEM):
                    cp.start()
        elif op[0] == "T":
            _, j0, j1, k0, k1 = op
            for j in range(j0, j1):
                t = load_k("w1", j, j + 1, k0, k1).T
                for k in range(k0, k1):
                    buf[w1t_block(j, k)] = t[:, KP[k] - KP[k0]:KP[k + 1] - KP[k0]]
        elif op[0] == "mm1":
            _, i0, i1, j0, j1, k0, k1 = op
            lhs = jnp.concatenate(
                [jnp.concatenate([buf[w1t_block(j, k)] for k in range(k0, k1)], axis=1)
                 for j in range(j0, j1)], axis=0)
            h = jnp.dot(lhs, load_k("x", i0, i1, k0, k1), preferred_element_type=jnp.float32)
            done = k_done.get((i0, j0), 0)
            if done:
                h = h + gather(hid, i0, i1, j0, j1)
            done += k1 - k0
            if done == NK:
                h = _silu(h).astype(jnp.bfloat16)
            for i in range(i0, i1):
                for j in range(j0, j1):
                    hid[i, j] = h[(j - j0) * U:(j - j0 + 1) * U, (i - i0) * U:(i - i0 + 1) * U]
                    k_done[i, j] = done
        elif op[0] == "pin":
            buf[0:16, cols("pin", 0, 1)] = hid[op[1], op[2]][U - 16:U].astype(buf.dtype)
        else:
            _, i0, i1, r0, r1 = op
            o = jnp.dot(buf[r0:r1, cols("w2", 0, NF)], gather(hid, i0, i1, 0, NF),
                        preferred_element_type=jnp.float32)
            o_buf[r0:r1, i0 * U:i1 * U] = o.astype(o_buf.dtype)
            cp = pltpu.make_async_copy(o_buf.at[r0:r1, i0 * U:i1 * U],
                                       oT_hbm.at[r0:r1, i0 * U:i1 * U], sems.at[0])
            cp.start()
            out_copies.append(cp)
    for cp in out_copies:
        cp.wait()


@jax.jit
def pallas_standalone__dense_activation_silu__prompt_kernel(
    x: jax.Array,
    w1: jax.Array,
    w2: jax.Array,
):
    assert x.shape == (1, S, D) and w1.shape == (D, F) and w2.shape == (F, D)
    assert x.dtype == w1.dtype == w2.dtype == jnp.bfloat16
    flags = {"XLA_TPU_RESCHEDULE_DMA_DONES": True} if jax.__version_info__ >= (0, 12) else None
    out_t = pl.pallas_call(
        _kernel,
        in_specs=[pl.BlockSpec(memory_space=pl.ANY)] * 3,
        out_specs=pl.BlockSpec(memory_space=pl.ANY),
        out_shape=jax.ShapeDtypeStruct((D, S), x.dtype),
        scratch_shapes=[
            pltpu.VMEM((D, _BUF_UNITS * U), jnp.bfloat16),
            pltpu.VMEM((D, (NS | 1) * U), jnp.bfloat16),
            pltpu.SemaphoreType.DMA((NSEM,)),
        ],
        compiler_params=pltpu.CompilerParams(vmem_limit_bytes=100 * 1024 * 1024, flags=flags),
    )(x.reshape(S, D).T, w1, w2.T)
    return out_t.T.reshape(1, S, D)
```

```python
import jax
import jax.numpy as jnp
import jax.experimental.pallas as pl
import jax.experimental.pallas.tpu as pltpu

U = 128
D, F, S = 448, 1792, 2048
NF, NS = F // U, S // U
NK = 4
KB = (0, 128, 256, 384, 448)
KP = (0, 128, 256, 384, 512)
REM, MAIN, ALL = (3, 4), (0, 3), (0, 4)
NSEM = 3

_GROUPS = (
    (("w1", 0, 4, *REM),),
    (("x", 0, 4, *REM),),
    (("x", 4, 8, *REM), ("w1", 4, 8, *REM)),
    (("x", 8, NS, *REM),),
    (("w1", 0, 4, *MAIN), ("x", 0, 4, *MAIN)),
    (("w1", 4, 8, *MAIN), ("x", 4, 8, *MAIN)),
    (("w1", 8, NF, *ALL), ("x", 8, NS, *MAIN)),
    (("w2", 0, NF, *ALL),),
)

_PROG = (
    ("wait", 0), ("T", 0, 4, *REM),
    ("wait", 1), ("mm1", 0, 4, 0, 4, *REM), ("pin", 3, 0),
    ("wait", 2), ("T", 4, 8, *REM), ("mm1", 4, 8, 0, 4, *REM), ("mm1", 0, 8, 4, 8, *REM),
    ("pin", 7, 5),
    ("wait", 3), ("mm1", 8, NS, 0, 8, *REM), ("pin", NS - 1, 2),
    ("wait", 4), ("T", 0, 4, *MAIN), ("mm1", 0, 4, 0, 4, *MAIN),
    ("wait", 5), ("T", 4, 8, *MAIN), ("mm1", 4, 8, 0, 4, *MAIN),
    ("wait", 6), ("T", 8, NF, *ALL), ("mm1", 0, 8, 4, 8, *MAIN), ("mm1", 8, NS, 0, 8, *MAIN),
    ("mm1", 0, NS, 8, NF, *ALL),
    ("wait", 7),
    ("mm2", 0, 4, 0, D), ("mm2", 4, 8, 0, D), ("mm2", 8, 12, 0, D), ("mm2", 12, 14, 0, D),
    ("mm2", 14, 15, 0, D), ("mm2", 15, NS, 0, D // 2), ("mm2", 15, NS, D // 2, D),
)
_N_HEAD = 2

_BASE = {"x": 0, "w1": NS, "w2": NS + NF, "w1T": NS + 2 * NF}
_BASE["pin"] = _BASE["w1T"] + (NK * NF + 2) // 3
_BUF_UNITS = (_BASE["pin"] + 1) | 1


_LOG2_E = 1.4426950408889634


def _silu(h):
    return h * pltpu.reciprocal(1.0 + jnp.exp2(h * -_LOG2_E), approx=True)


def _kernel(xT_hbm, w1_hbm, w2T_hbm, oT_hbm, buf, o_buf, sems):
    hbm = {"x": xT_hbm, "w1": w1_hbm, "w2": w2T_hbm}

    def cols(name, u0, u1):
        return slice((_BASE[name] + u0) * U, (_BASE[name] + u1) * U)

    def w1t_block(j, k):
        unit, slot = divmod(k * NF + j, 3)
        return slice(slot * U, (slot + 1) * U), cols("w1T", unit, unit + 1)

    def load_k(name, u0, u1, k0, k1):
        val = buf[KB[k0]:KB[k1], cols(name, u0, u1)]
        if k1 == NK:
            zeros = jnp.zeros((KP[NK] - D, val.shape[1]), val.dtype)
            val = jnp.concatenate([val, zeros], axis=0)
        return val

    def in_copies(g):
        return [
            pltpu.make_async_copy(
                hbm[name].at[KB[k0]:KB[k1], u0 * U:u1 * U],
                buf.at[KB[k0]:KB[k1], cols(name, u0, u1)],
                sems.at[g % NSEM])
            for name, u0, u1, k0, k1 in _GROUPS[g]
        ]

    def gather(tiles, i0, i1, j0, j1):
        return jnp.concatenate(
            [jnp.concatenate([tiles[i, j] for i in range(i0, i1)], axis=1)
             for j in range(j0, j1)], axis=0)

    for g in range(NSEM):
        for cp in in_copies(g):
            cp.start()

    def run(prog):
        hid = {}
        k_done = {}
        out_copies = []
        for op in prog:
            if op[0] == "wait":
                g = op[1]
                for cp in in_copies(g):
                    cp.wait()
                if g + NSEM < len(_GROUPS):
                    for cp in in_copies(g + NSEM):
                        cp.start()
            elif op[0] == "T":
                _, j0, j1, k0, k1 = op
                for j in range(j0, j1):
                    t = load_k("w1", j, j + 1, k0, k1).T
                    for k in range(k0, k1):
                        buf[w1t_block(j, k)] = t[:, KP[k] - KP[k0]:KP[k + 1] - KP[k0]]
            elif op[0] == "mm1":
                _, i0, i1, j0, j1, k0, k1 = op
                lhs = jnp.concatenate(
                    [jnp.concatenate([buf[w1t_block(j, k)] for k in range(k0, k1)], axis=1)
                     for j in range(j0, j1)], axis=0)
                h = jnp.dot(lhs, load_k("x", i0, i1, k0, k1), preferred_element_type=jnp.float32)
                done = k_done.get((i0, j0), 0)
                if done:
                    h = h + gather(hid, i0, i1, j0, j1)
                done += k1 - k0
                if done == NK:
                    h = _silu(h).astype(jnp.bfloat16)
                for i in range(i0, i1):
                    for j in range(j0, j1):
                        hid[i, j] = h[(j - j0) * U:(j - j0 + 1) * U, (i - i0) * U:(i - i0 + 1) * U]
                        k_done[i, j] = done
            elif op[0] == "pin":
                buf[0:16, cols("pin", 0, 1)] = hid[op[1], op[2]][U - 16:U].astype(buf.dtype)
            else:
                _, i0, i1, r0, r1 = op
                o = jnp.dot(buf[r0:r1, cols("w2", 0, NF)], gather(hid, i0, i1, 0, NF),
                            preferred_element_type=jnp.float32)
                o_buf[r0:r1, i0 * U:i1 * U] = o.astype(o_buf.dtype)
                cp = pltpu.make_async_copy(o_buf.at[r0:r1, i0 * U:i1 * U],
                                           oT_hbm.at[r0:r1, i0 * U:i1 * U], sems.at[0])
                cp.start()
                out_copies.append(cp)
        for cp in out_copies:
            cp.wait()

    def main(trip):
        run(_PROG[_N_HEAD:])
        return trip + 1

    run(_PROG[:_N_HEAD])
    jax.lax.while_loop(lambda trip: trip < 1, main, 0)


@jax.jit
def pallas_standalone__dense_activation_silu__prompt_kernel(
    x: jax.Array,
    w1: jax.Array,
    w2: jax.Array,
):
    assert x.shape == (1, S, D) and w1.shape == (D, F) and w2.shape == (F, D)
    assert x.dtype == w1.dtype == w2.dtype == jnp.bfloat16
    flags = {"XLA_TPU_RESCHEDULE_DMA_DONES": True} if jax.__version_info__ >= (0, 12) else None
    out_t = pl.pallas_call(
        _kernel,
        in_specs=[pl.BlockSpec(memory_space=pl.ANY)] * 3,
        out_specs=pl.BlockSpec(memory_space=pl.ANY),
        out_shape=jax.ShapeDtypeStruct((D, S), x.dtype),
        scratch_shapes=[
            pltpu.VMEM((D, _BUF_UNITS * U), jnp.bfloat16),
            pltpu.VMEM((D, (NS | 1) * U), jnp.bfloat16),
            pltpu.SemaphoreType.DMA((NSEM,)),
        ],
        compiler_params=pltpu.CompilerParams(vmem_limit_bytes=64 * 1024 * 1024, flags=flags),
    )(x.reshape(S, D).T, w1, w2.T)
    return out_t.T.reshape(1, S, D)
```
